```python
import os as _os
_os.environ.setdefault("JAX_PLATFORMS", "cpu")
import jax
import jax.numpy as jnp

def _softmax(x, axis=-1):
    return jax.nn.softmax(x, axis=axis)
def _gelu(x):
    return jax.nn.gelu(x, approximate=True)
def _silu(x):
    return jax.nn.silu(x)
def _sigmoid(x):
    return jax.nn.sigmoid(x)
def _layernorm(x, axis=-1, eps=1e-5):
    m = jnp.mean(x, axis=axis, keepdims=True)
    v = jnp.var(x, axis=axis, keepdims=True)
    return (x - m) / jnp.sqrt(v + eps)
def _scatter_add(tgt, idx, src, axis=0):
    return tgt.at[idx].add(src)
def _segment_sum(src, seg, n):
    return jax.ops.segment_sum(src, seg, n)
class _Rng:
    def __init__(self, key):
        self._k = key
    def _next(self):
        self._k, sub = jax.random.split(self._k)
        return sub
    def normal(self, shape):
        return jax.random.normal(self._next(), shape, dtype=jnp.bfloat16)
    def randint(self, lo, hi, shape):
        return jax.random.randint(self._next(), shape, lo, hi, dtype=jnp.int32)
    def uniform(self, shape, lo=0.0, hi=1.0):
        return jax.random.uniform(self._next(), shape, jnp.bfloat16, lo, hi)
    def permutation(self, n):
        return jax.random.permutation(self._next(), n)


kernel_name = 'concat_heads__sliding_block__ssm_conv_s4__prompt'

def setup_inputs():
    _rng = _Rng(jax.random.key(int.from_bytes(__import__("os").urandom(4), "little")))
    _w = (lambda a: (lambda t: t.astype(jnp.bfloat16) if jnp.issubdtype(t.dtype, jnp.floating) else t)(jnp.asarray(a)))
    def _A_setup():
        B, S, D = 1, 2048, 512
        return {
            "x": _w((lambda *s: _rng.normal(s) * 0.2)(B, S, D)),
            "wqkv": _w((lambda *s: _rng.normal(s) * 0.2)(D, 3 * D)),
            "wo": _w((lambda *s: _rng.normal(s) * 0.05)(D, D)),
        }
    _A_in = _A_setup()

    def _B_setup():
        B, L, D, N = 1, 2048, 512, 128
        A_re = -jnp.exp((lambda *s: _rng.normal(s) * 0.8)(D, N))
        A_im = jnp.pi * (lambda *s: _rng.normal(s) * 0.8)(D, N)
        B_re = (lambda *s: _rng.normal(s) * 0.8)(D, N)
        B_im = (lambda *s: _rng.normal(s) * 0.8)(D, N)
        C_re = (lambda *s: _rng.normal(s) * 0.8)(D, N)
        C_im = (lambda *s: _rng.normal(s) * 0.8)(D, N)
        log_dt = (lambda *s: _rng.normal(s) * 0.8)(D) * 0.5 - 4.0
        Dskip = (lambda *s: _rng.normal(s) * 0.05)(D)
        return {
            "u": _w((lambda *s: _rng.normal(s) * 0.05)(B, L, D)),
            "A_re": _w(A_re),
            "A_im": _w(A_im),
            "B_re": _w(B_re),
            "B_im": _w(B_im),
            "C_re": _w(C_re),
            "C_im": _w(C_im),
            "log_dt": _w(log_dt),
            "Dskip": _w(Dskip),
        }
    _B_in = _B_setup()

    return {
        "A_x": _A_in["x"],
        "A_wqkv": _A_in["wqkv"],
        "A_wo": _A_in["wo"],
        "B_u": _B_in["u"],
        "B_A_re": _B_in["A_re"],
        "B_A_im": _B_in["A_im"],
        "B_B_re": _B_in["B_re"],
        "B_B_im": _B_in["B_im"],
        "B_C_re": _B_in["C_re"],
        "B_C_im": _B_in["C_im"],
        "B_log_dt": _B_in["log_dt"],
        "B_Dskip": _B_in["Dskip"],
    }

def reference(A_x, A_wqkv, A_wo, B_u, B_A_re, B_A_im, B_B_re, B_B_im, B_C_re, B_C_im, B_log_dt, B_Dskip):
    def _A_ref(x, wqkv, wo):
        B, S, D = x.shape
        H = 32; Dh = D // H; W = 256
        qkv = (lambda x, *d: x.transpose(*d))((x @ wqkv).reshape(B, S, 3, H, Dh), 2, 0, 3, 1, 4)
        q, k, v = qkv[0], qkv[1], qkv[2]
        scores = jnp.einsum("bhqd,bhkd->bhqk", q, k) * (Dh ** -0.5)
        idx = jnp.arange(S)
        mask = (idx[:, None] - idx[None, :] >= 0) & (idx[:, None] - idx[None, :] < W)
        scores = jnp.where(mask[None, None], scores, -1e9)
        p = _softmax(scores, axis=-1)
        o = jnp.einsum("bhqk,bhkd->bhqd", p, v)
        return (lambda x, *d: x.transpose(*d))(o, 0, 2, 1, 3).reshape(B, S, D) @ wo

    def _B_ref(u, A_re, A_im, B_re, B_im, C_re, C_im, log_dt, Dskip):
        Bsz, L, D = u.shape
        dt = jnp.exp(log_dt)[:, None]
        A = A_re + 1j * A_im
        Bc = B_re + 1j * B_im
        Cc = C_re + 1j * C_im
        logdA = dt * A
        dB = dt * Bc
        l = (lambda x, dt: x.astype(dt))(jnp.arange(L), A_re.dtype)
        P = jnp.exp(logdA[:, :, None] * l[None, None, :])
        K = jnp.einsum("dn,dnl,dn->dl", Cc, P, dB).real
        L2 = 2 * L
        Kp = jnp.pad(K, ((0, 0), (0, L)))
        up = (lambda x, *d: x.transpose(*d))(u, 0, 2, 1)
        up = jnp.pad(up, ((0, 0), (0, 0), (0, L)))
        Kf = (lambda x, axes=(-2,-1): jnp.fft.rfft2(x.astype(jnp.float32), axes=axes))(Kp[:, None, :], axes=(-2, -1))
        Uf = (lambda x, axes=(-2,-1): jnp.fft.rfft2(x.astype(jnp.float32), axes=axes))(up[:, :, None, :], axes=(-2, -1))
        Yf = Uf * Kf[None, :, :, :]
        y = (lambda x, s, axes=(-2,-1): jnp.fft.irfft2(x, s=s, axes=axes).astype(jnp.bfloat16))(Yf, (1, L2), axes=(-2, -1))[:, :, 0, :L]
        y = (lambda x, *d: x.transpose(*d))(y, 0, 2, 1) + u * Dskip[None, None, :]
        return y

    a = _A_ref(A_x, A_wqkv, A_wo)
    b = _B_ref(B_u, B_A_re, B_A_im, B_B_re, B_B_im, B_C_re, B_C_im, B_log_dt, B_Dskip)
    return jnp.concatenate([a, b], axis=-1)
```

```python
import jax
import jax.numpy as jnp
import numpy as np
import ml_dtypes
import jax.experimental.pallas as pl
import jax.experimental.pallas.tpu as pltpu

f32 = jnp.float32
bf = jnp.bfloat16

S = 2048
DM = 512
NH, DH, WIN = 32, 16, 256
TQ = 128
NQ = S // TQ
NST = 128
NF = 2 * S
NG = DM // 128
R1 = 72
RC = 80

_LO_SET = list(range(16)) + list(range(16, 32, 2)) + list(range(32, 64, 4)) + list(range(64, 128, 8))
_IDX = {x: i for i, x in enumerate(_LO_SET)}
_NLO = len(_LO_SET)
_NT = _NLO + 40
for _k, _x in enumerate([128, 256, 512, 1024]):
    _IDX[_x] = _NT + _k
_NTALL = _NT + 4
_ANCH = (0, 4, 8)


def _hi_idx(r, i):
    return _NLO + [0, 16, 24, 32][r] + i


def _rows_pattern(step, nrows):
    out = []
    for rho in range(nrows):
        q, rem = divmod(rho, step)
        if 2 * rem < step:
            v = q
        elif 2 * rem > step:
            v = q + 1
        else:
            v = q if q % 2 == 0 else q + 1
        out.append(v)
    return out


def _assemble(rows, pat):
    pieces = []
    k = 0
    while k < len(pat):
        k2 = k
        while k2 < len(pat) and pat[k2] == pat[k]:
            k2 += 1
        pieces.append(jnp.broadcast_to(rows[pat[k]], (k2 - k, 128)) if k2 - k > 1 else rows[pat[k]])
        k = k2
    return jnp.concatenate(pieces, axis=0)


def _split_np(F):
    Fh = F.astype(np.float32).astype(ml_dtypes.bfloat16)
    Fl = (F - Fh.astype(np.float64)).astype(np.float32).astype(ml_dtypes.bfloat16)
    return Fh, Fl


def _make_dft_consts():
    k1 = np.arange(33)
    F1 = np.zeros((64, R1, 96), ml_dtypes.bfloat16)
    G = np.zeros((64, 32, 3 * RC), ml_dtypes.bfloat16)
    for n2 in range(64):
        n = 64 * np.arange(32) + n2
        ph = -2 * np.pi * np.outer(k1, n) / NF
        M = np.zeros((R1, 32))
        M[0:33] = np.cos(ph)
        M[33:66] = np.sin(ph)
        h, l = _split_np(M)
        F1[n2] = np.concatenate([h, l, h], 1)
        ph = 2 * np.pi * np.outer(n, k1) / NF
        w = np.full(33, 2.0)
        w[0] = 1
        w[32] = 1
        w /= NF
        M = np.zeros((32, RC))
        M[:, 0:33] = w * np.cos(ph)
        M[:, 40:73] = -w * np.sin(ph)
        h, l = _split_np(M)
        G[n2] = np.concatenate([h, l, h], 1)
    n2k2 = np.outer(np.arange(64), np.arange(64))
    C64 = np.cos(2 * np.pi * n2k2 / 64)
    S64 = -np.sin(2 * np.pi * n2k2 / 64)
    h, l = _split_np(np.block([[C64, -S64], [S64, C64]]))
    F2 = np.concatenate([h, l, h], 1)
    h, l = _split_np(np.block([[C64, S64], [-S64, C64]]))
    F2i = np.concatenate([h, l, h], 1)
    return F1, F2, F2i, G


_DFT_CONSTS = _make_dft_consts()


def _split3(x):
    xh = x.astype(bf)
    xl = (x - xh.astype(f32)).astype(bf)
    return jnp.concatenate([xh, xh, xl], axis=0)


_T_ROWS = 2 * _NTALL * NST
_BU0 = 0
_BK0 = _BU0 + 64 * R1
_CS0 = _BK0 + 64 * R1
_YS0 = _CS0 + 64 * RC
assert _YS0 + S <= _T_ROWS


def _kernel(x_ref, wqkv_ref, wo_ref, u_ref, are_ref, aim_ref, bre_ref, bim_ref, cre_ref, cim_ref,
            ldt_ref, dsk_ref, F1_ref, F2_ref, F2i_ref, G_ref,
            out_ref,
            q_scr, k_scr, vT_scr, OT_scr, S_scr, T, P_scr, Ks, u32):
    dt = jnp.exp(ldt_ref[...].astype(f32)).astype(bf).astype(f32)

    def tr(ref):
        return ref[...].astype(f32).T

    ar = tr(are_ref) * dt
    ai = tr(aim_ref) * dt
    dBr = tr(bre_ref) * dt
    dBi = tr(bim_ref) * dt
    Cr = tr(cre_ref)
    Ci = tr(cim_ref)
    P_scr[0] = ar
    P_scr[1] = ai
    P_scr[2] = Cr * dBr - Ci * dBi
    P_scr[3] = Cr * dBi + Ci * dBr

    def tables_slice(it, carry):
        lg = it // (NST // 8)
        s = it % (NST // 8)
        lanes = pl.ds(pl.multiple_of(lg * 128, 128), 128)
        prow = pl.ds(pl.multiple_of(s * 8, 8), 8)

        def trow(e):
            return pl.ds(pl.multiple_of(e * NST + s * 8, 8), 8)

        def st(idx, v):
            T[lg, trow(2 * idx), :] = v[0]
            T[lg, trow(2 * idx + 1), :] = v[1]

        def ld(idx):
            return T[lg, trow(2 * idx), :], T[lg, trow(2 * idx + 1), :]

        def cmul(a, b):
            return a[0] * b[0] - a[1] * b[1], a[0] * b[1] + a[1] * b[0]

        ar_s = P_scr[0, prow, lanes]
        ai_s = P_scr[1, prow, lanes]
        st(_IDX[0], (jnp.ones((8, 128), f32), jnp.zeros((8, 128), f32)))
        e = None
        for b in range(11):
            if b in _ANCH:
                xx = float(2 ** b)
                m = jnp.exp(ar_s * xx)
                th = ai_s * xx
                e = (m * jnp.cos(th), m * jnp.sin(th))
            else:
                e = (e[0] * e[0] - e[1] * e[1], 2.0 * e[0] * e[1])
            st(_IDX[2 ** b], e)
        for xv in _LO_SET:
            if xv == 0 or (xv & (xv - 1)) == 0:
                continue
            low = xv & (-xv)
            st(_IDX[xv], cmul(ld(_IDX[xv - low]), ld(_IDX[low])))
        st(_hi_idx(0, 0), (P_scr[2, prow, lanes], P_scr[3, prow, lanes]))
        for i in range(1, 16):
            low = i & (-i)
            st(_hi_idx(0, i), cmul(ld(_hi_idx(0, i - low)), ld(_IDX[16 * low])))

        def h_of(xv):
            if xv < 256:
                return _hi_idx(0, xv // 16)
            if xv < 512:
                return _hi_idx(1, (xv - 256) // 32)
            return _hi_idx(2, (xv - 512) // 64)

        for r in (1, 2, 3):
            base = 128 << r
            st16 = 16 << r
            for i in range(8):
                st(_hi_idx(r, i), cmul(ld(h_of(st16 * i)), ld(_IDX[base])))
        return carry

    jax.lax.fori_loop(0, NG * (NST // 8), tables_slice, 0)

    def kgen_unit(lg, r, ia, jh, A=4):
        step = 1 << r
        B = 8 if r == 0 else 9
        lidx = [jnp.where(jh == 0, _IDX[step * j], _IDX[step * (8 + j)]) for j in range(B)]
        hidx = [_hi_idx(r, 0) + A * ia + a for a in range(A)]

        def tl(e, s):
            return T[lg, pl.ds(pl.multiple_of(e * NST + s * 8, 8), 8), :]

        accs = [[None] * B for _ in range(A)]
        for s in range(NST // 8):
            hs = [(tl(2 * h, s), tl(2 * h + 1, s)) for h in hidx]
            for q in range(B):
                lr = tl(2 * lidx[q], s)
                li = tl(2 * lidx[q] + 1, s)
                for a in range(A):
                    t = hs[a][0] * lr - hs[a][1] * li
                    accs[a][q] = t if s == 0 else accs[a][q] + t
        tot = accs[0][0]
        for a in range(A):
            for q in range(B):
                if a or q:
                    tot = tot + accs[a][q]
        never = jh < 0
        accs = [[jnp.where(never, tot, accs[a][q]) for q in range(B)] for a in range(A)]
        base = 0 if r == 0 else (128 << r)
        pat = _rows_pattern(step, 8 * step)
        for a in range(A):
            rows = [jnp.sum(v, axis=0, keepdims=True) for v in accs[a]]
            l0 = pl.multiple_of(base + 16 * step * (A * ia + a) + 8 * step * jh, 8)
            Ks[lg, pl.ds(l0, 8 * step), :] = _assemble(rows, pat)

    def kmain0(it, carry):
        kgen_unit(it // 8, 0, (it // 2) % 4, it % 2)
        return carry

    jax.lax.fori_loop(0, 32, kmain0, 0)
    for r in (1, 2, 3):
        def kmainr(it, carry, r=r):
            kgen_unit(it // 4, r, (it // 2) % 2, it % 2)
            return carry

        jax.lax.fori_loop(0, 16, kmainr, 0)

    k_scr[0:256, :] = jnp.zeros((256, DM), bf)
    vT_scr[:, 0:256] = jnp.zeros((DM, 256), bf)
    CH = 256
    for c in range(S // CH):
        xc = x_ref[c * CH:(c + 1) * CH, :]
        qk = jnp.dot(xc, wqkv_ref[:, 0:2 * DM], preferred_element_type=f32)
        q_scr[c * CH:(c + 1) * CH, :] = (qk[:, :DM] * (DH ** -0.5)).astype(bf)
        k_scr[256 + c * CH:256 + (c + 1) * CH, :] = qk[:, DM:].astype(bf)
        vT = jax.lax.dot_general(wqkv_ref[:, 2 * DM:3 * DM], xc, (((0,), (1,)), ((), ())),
                                 preferred_element_type=f32)
        vT_scr[:, 256 + c * CH:256 + (c + 1) * CH] = vT.astype(bf)

    row = jax.lax.broadcasted_iota(jnp.int32, (TQ, TQ), 0)
    col = jax.lax.broadcasted_iota(jnp.int32, (TQ, TQ), 1)
    tri = row <= col
    lane_head = col // DH

    def qk_unit(i, g, slot):
        r0 = pl.multiple_of(i * TQ, TQ)
        q_blk = q_scr[pl.ds(r0, TQ), g * 128:(g + 1) * 128]
        k_rows = k_scr[pl.ds(r0, 3 * TQ), g * 128:(g + 1) * 128]
        qm = jnp.concatenate(
            [jnp.where(lane_head == hh, q_blk, jnp.zeros_like(q_blk)) for hh in range(8)], axis=0)
        S_scr[slot] = jax.lax.dot_general(k_rows, qm, (((1,), (1,)), ((), ())),
                                          preferred_element_type=f32)

    def softpv_unit(i, g, slot):
        r0 = pl.multiple_of(i * TQ, TQ)
        for hh in range(8):
            h = g * 8 + hh
            U = S_scr[slot, 0:TQ, hh * 128:(hh + 1) * 128]
            M = S_scr[slot, TQ:2 * TQ, hh * 128:(hh + 1) * 128]
            Dg = S_scr[slot, 2 * TQ:3 * TQ, hh * 128:(hh + 1) * 128]
            neg = jnp.full((TQ, TQ), -1e9, f32)
            U = jnp.where(i >= 2, U, neg)
            M = jnp.where(i >= 1, M, neg)
            C = jnp.where(tri, Dg, U)
            m = jnp.max(jnp.maximum(C, M), axis=0, keepdims=True)
            PC = jnp.exp(C - m)
            PM = jnp.exp(M - m)
            l = jnp.sum(PC + PM, axis=0, keepdims=True)
            PD = jnp.where(tri, PC, 0.0)
            PU = PC - PD
            PT = jnp.concatenate([PU, PM, PD], axis=0).astype(bf)
            vh = vT_scr[h * DH:(h + 1) * DH, pl.ds(r0, 3 * TQ)]
            oT = jnp.dot(vh, PT, preferred_element_type=f32)
            OT_scr[h * DH:(h + 1) * DH, pl.ds(r0, TQ)] = (oT / l).astype(bf)

    qk_unit(0, 0, 0)

    def qblock(i, carry):
        qk_unit(i, 1, 1)
        softpv_unit(i, 0, 0)
        qk_unit(i, 2, 0)
        softpv_unit(i, 1, 1)
        qk_unit(i, 3, 1)
        softpv_unit(i, 2, 0)
        qk_unit(jnp.minimum(i + 1, NQ - 1), 0, 0)
        softpv_unit(i, 3, 1)
        return carry

    jax.lax.fori_loop(0, NQ, qblock, 0)

    for c in range(S // CH):
        o = jax.lax.dot_general(OT_scr[:, c * CH:(c + 1) * CH], wo_ref[...], (((0,), (0,)), ((), ())),
                                preferred_element_type=f32)
        out_ref[c * CH:(c + 1) * CH, 0:DM] = o.astype(bf)

    for g in range(NG):
        u32[g] = u_ref[:, g * 128:(g + 1) * 128].astype(f32)
    zero8 = jnp.zeros((8, 128), f32)

    def s1(n2, carry):
        F = F1_ref[n2]
        r0 = pl.multiple_of(n2 * R1, 8)
        c0 = pl.multiple_of(n2 * RC, 8)
        for g in range(NG):
            xu = u32[g, pl.ds(n2, 32, stride=64), :].astype(bf)
            T[g, pl.ds(_BU0 + r0, R1), :] = jnp.dot(F[:, 0:64], jnp.concatenate([xu, xu], axis=0),
                                                    preferred_element_type=f32)
            T[g, pl.ds(_BK0 + r0, R1), :] = jnp.dot(F, _split3(Ks[g, pl.ds(n2, 32, stride=64), :]),
                                                    preferred_element_type=f32)
            T[g, pl.ds(_CS0 + c0 + 32, 8), :] = zero8
            T[g, pl.ds(_CS0 + c0 + 72, 8), :] = zero8
        return carry

    jax.lax.fori_loop(0, 64, s1, 0, unroll=4)

    def s2(k1, carry):
        F2 = F2_ref[...]
        F2i = F2i_ref[...]
        Xs = []
        for g in range(NG):
            iu = jnp.concatenate([T[g, pl.ds(_BU0 + k1, 64, stride=R1), :],
                                  T[g, pl.ds(_BU0 + 33 + k1, 64, stride=R1), :]], axis=0)
            Xu = jnp.dot(F2, _split3(iu), preferred_element_type=f32)
            ik = jnp.concatenate([T[g, pl.ds(_BK0 + k1, 64, stride=R1), :],
                                  T[g, pl.ds(_BK0 + 33 + k1, 64, stride=R1), :]], axis=0)
            Xk = jnp.dot(F2, _split3(ik), preferred_element_type=f32)
            Xs.append((Xu, Xk))
        for g in range(NG):
            Xu, Xk = Xs[g]
            ur, ui, kr, ki = Xu[0:64], Xu[64:128], Xk[0:64], Xk[64:128]
            Y = jnp.concatenate([ur * kr - ui * ki, ur * ki + ui * kr], axis=0)
            Cv = jnp.dot(F2i, _split3(Y), preferred_element_type=f32)
            T[g, pl.ds(_CS0 + k1, 64, stride=RC), :] = Cv[0:64]
            T[g, pl.ds(_CS0 + 40 + k1, 64, stride=RC), :] = Cv[64:128]
        return carry

    jax.lax.fori_loop(0, 33, s2, 0, unroll=3)

    def s3(n2, carry):
        Gm = G_ref[n2]
        for g in range(NG):
            inp = T[g, pl.ds(pl.multiple_of(_CS0 + n2 * RC, 8), RC), :]
            T[g, pl.ds(_YS0 + n2, 32, stride=64), :] = jnp.dot(Gm, _split3(inp), preferred_element_type=f32)
        return carry

    jax.lax.fori_loop(0, 64, s3, 0, unroll=4)

    for g in range(NG):
        yb = T[g, _YS0:_YS0 + S, :].astype(bf).astype(f32)
        sk = (u32[g] * dsk_ref[:, g * 128:(g + 1) * 128].astype(f32)).astype(bf).astype(f32)
        out_ref[:, DM + g * 128:DM + (g + 1) * 128] = (yb + sk).astype(bf)


@jax.jit
def pallas_concat_heads__sliding_block__ssm_conv_s4__prompt_kernel(
    A_x: jax.Array,
    A_wqkv: jax.Array,
    A_wo: jax.Array,
    B_u: jax.Array,
    B_A_re: jax.Array,
    B_A_im: jax.Array,
    B_B_re: jax.Array,
    B_B_im: jax.Array,
    B_C_re: jax.Array,
    B_C_im: jax.Array,
    B_log_dt: jax.Array,
    B_Dskip: jax.Array,
):
    F1, F2, F2i, G = [jnp.asarray(c) for c in _DFT_CONSTS]
    out = pl.pallas_call(
        _kernel,
        out_shape=jax.ShapeDtypeStruct((S, 2 * DM), bf),
        scratch_shapes=[
            pltpu.VMEM((S, DM), bf),
            pltpu.VMEM((S + 256, DM), bf),
            pltpu.VMEM((DM, S + 256), bf),
            pltpu.VMEM((DM, S), bf),
            pltpu.VMEM((2, 3 * TQ, 8 * TQ), f32),
            pltpu.VMEM((NG, _T_ROWS, 128), f32),
            pltpu.VMEM((4, NST, DM), f32),
            pltpu.VMEM((NG, S, 128), f32),
            pltpu.VMEM((NG, S, 128), f32),
        ],
        compiler_params=pltpu.CompilerParams(vmem_limit_bytes=120 * 1024 * 1024),
    )(A_x.reshape(S, DM), A_wqkv, A_wo, B_u.reshape(S, DM),
      B_A_re, B_A_im, B_B_re, B_B_im, B_C_re, B_C_im,
      B_log_dt.reshape(1, DM), B_Dskip.reshape(1, DM), F1, F2, F2i, G)
    return out.reshape(1, S, 2 * DM)
```

```python
import jax
import jax.numpy as jnp
import numpy as np
import ml_dtypes
import jax.experimental.pallas as pl
import jax.experimental.pallas.tpu as pltpu

f32 = jnp.float32
bf = jnp.bfloat16

S = 2048
DM = 512
DH = 16
LOG2E = 1.4426950408889634
TQ = 128
NQ = S // TQ
NST = 128
NF = 2 * S
NG = DM // 128
R1 = 72
RC = 80

_LO_SET = list(range(16)) + list(range(16, 32, 2)) + list(range(32, 64, 4)) + list(range(64, 128, 8))
_IDX = {x: i for i, x in enumerate(_LO_SET)}
_NLO = len(_LO_SET)
_NT = _NLO + 40
for _k, _x in enumerate([128, 256, 512, 1024]):
    _IDX[_x] = _NT + _k
_NTALL = _NT + 4
_ANCH = (0, 4, 8)


def _hi_idx(r, i):
    return _NLO + [0, 16, 24, 32][r] + i


def _rows_pattern(step, nrows):
    out = []
    for rho in range(nrows):
        q, rem = divmod(rho, step)
        if 2 * rem < step:
            v = q
        elif 2 * rem > step:
            v = q + 1
        else:
            v = q if q % 2 == 0 else q + 1
        out.append(v)
    return out


def _assemble(rows, pat):
    pieces = []
    k = 0
    while k < len(pat):
        k2 = k
        while k2 < len(pat) and pat[k2] == pat[k]:
            k2 += 1
        pieces.append(jnp.broadcast_to(rows[pat[k]], (k2 - k, 128)) if k2 - k > 1 else rows[pat[k]])
        k = k2
    return jnp.concatenate(pieces, axis=0)


def _split_np(F):
    Fh = F.astype(np.float32).astype(ml_dtypes.bfloat16)
    Fl = (F - Fh.astype(np.float64)).astype(np.float32).astype(ml_dtypes.bfloat16)
    return Fh, Fl


def _make_dft_consts():
    k1 = np.arange(33)
    F1 = np.zeros((64, R1, 96), ml_dtypes.bfloat16)
    G = np.zeros((64, 32, 3 * RC), ml_dtypes.bfloat16)
    for n2 in range(64):
        n = 64 * np.arange(32) + n2
        ph = -2 * np.pi * np.outer(k1, n) / NF
        M = np.zeros((R1, 32))
        M[0:33] = np.cos(ph)
        M[33:66] = np.sin(ph)
        h, l = _split_np(M)
        F1[n2] = np.concatenate([h, l, h], 1)
        ph = 2 * np.pi * np.outer(n, k1) / NF
        w = np.full(33, 2.0)
        w[0] = 1
        w[32] = 1
        w /= NF
        M = np.zeros((32, RC))
        M[:, 0:33] = w * np.cos(ph)
        M[:, 40:73] = -w * np.sin(ph)
        h, l = _split_np(M)
        G[n2] = np.concatenate([h, l, h], 1)
    n2k2 = np.outer(np.arange(64), np.arange(64))
    C64 = np.cos(2 * np.pi * n2k2 / 64)
    S64 = -np.sin(2 * np.pi * n2k2 / 64)
    h, l = _split_np(np.block([[C64, -S64], [S64, C64]]))
    F2 = np.concatenate([h, l, h], 1)
    h, l = _split_np(np.block([[C64, S64], [-S64, C64]]))
    F2i = np.concatenate([h, l, h], 1)
    return F1, F2, F2i, G


_DFT_CONSTS = _make_dft_consts()


def _sincos(x):
    k = jnp.floor(x * 0.6366197723675814 + 0.5)
    r = ((x - k * 1.5703125) - k * 4.837512969970703125e-4) - k * 7.54978995489188216e-8
    z = r * r
    s = ((-1.9515295891e-4 * z + 8.3321608736e-3) * z - 1.6666654611e-1) * z * r + r
    c = ((2.443315711809948e-5 * z - 1.388731625493765e-3) * z + 4.166664568298827e-2) * z * z - 0.5 * z + 1.0
    q = k.astype(jnp.int32)
    swap = (q & 1) != 0
    sn = jnp.where(swap, c, s)
    cs = jnp.where(swap, s, c)
    sn = jnp.where((q & 2) != 0, -sn, sn)
    cs = jnp.where(((q + 1) & 2) != 0, -cs, cs)
    return sn, cs


def _split3(x):
    xh = x.astype(bf)
    xl = (x - xh.astype(f32)).astype(bf)
    return jnp.concatenate([xh, xh, xl], axis=0)


def _transpose8(vs):
    sub = jax.lax.broadcasted_iota(jnp.int32, (8, 128), 0)
    for sh in (4, 2, 1):
        low = (sub & sh) == 0
        new = list(vs)
        for a in range(8):
            if a & sh == 0:
                lo, hi = vs[a], vs[a + sh]
                new[a] = jnp.where(low, lo, pltpu.roll(hi, sh, 0))
                new[a + sh] = jnp.where(low, pltpu.roll(lo, 8 - sh, 0), hi)
        vs = new
    return vs


_T_ROWS = 2 * _NTALL * NST
_BU0 = 0
_BK0 = _BU0 + 64 * R1
assert _BK0 + 64 * R1 <= _T_ROWS


def _kernel(x_hbm, wqkv_hbm, wo_hbm, u_hbm, are_ref, aim_ref, bre_ref, bim_ref, cre_ref, cim_ref,
            ldt_ref, dsk_ref, F1_hbm, F2_hbm, F2i_hbm, G_hbm,
            out_hbm,
            q_scr, k_scr, vT_scr, OT_scr, S_scr, Mx_scr, T, P_scr, Ks, u32, Cs,
            x_ref, wqkv_ref, wo_ref, u_ref, F1_ref, F2_ref, F2i_ref, G_ref, outA, outB, in_sems, out_sems):
    in_pairs = [(x_hbm, x_ref), (wqkv_hbm, wqkv_ref), (u_hbm, u_ref), (F1_hbm, F1_ref), (F2_hbm, F2_ref),
                (F2i_hbm, F2i_ref), (G_hbm, G_ref), (wo_hbm, wo_ref)]
    in_copies = [pltpu.make_async_copy(src, dst, in_sems.at[j]) for j, (src, dst) in enumerate(in_pairs)]
    for cp in in_copies:
        cp.start()

    dt = jnp.exp(ldt_ref[...].astype(f32)).astype(bf).astype(f32)

    def tr(ref):
        return ref[...].astype(f32).T

    ar = tr(are_ref) * dt
    ai = tr(aim_ref) * dt
    dBr = tr(bre_ref) * dt
    dBi = tr(bim_ref) * dt
    Cr = tr(cre_ref)
    Ci = tr(cim_ref)
    P_scr[0] = ar
    P_scr[1] = ai
    P_scr[2] = Cr * dBr - Ci * dBi
    P_scr[3] = Cr * dBi + Ci * dBr

    def tables_slice(it, carry):
        lg = it // (NST // 8)
        s = it % (NST // 8)
        lanes = pl.ds(pl.multiple_of(lg * 128, 128), 128)
        prow = pl.ds(pl.multiple_of(s * 8, 8), 8)

        def trow(e):
            return pl.ds(pl.multiple_of(e * NST + s * 8, 8), 8)

        def st(idx, v):
            T[lg, trow(2 * idx), :] = v[0]
            T[lg, trow(2 * idx + 1), :] = v[1]

        def ld(idx):
            return T[lg, trow(2 * idx), :], T[lg, trow(2 * idx + 1), :]

        def cmul(a, b):
            return a[0] * b[0] - a[1] * b[1], a[0] * b[1] + a[1] * b[0]

        ar_s = P_scr[0, prow, lanes]
        ai_s = P_scr[1, prow, lanes]
        st(_IDX[0], (jnp.ones((8, 128), f32), jnp.zeros((8, 128), f32)))
        e = None
        for b in range(11):
            if b in _ANCH:
                xx = float(2 ** b)
                m = jnp.exp(ar_s * xx)
                th = ai_s * xx
                sn, cs = _sincos(th)
                e = (m * cs, m * sn)
            else:
                e = (e[0] * e[0] - e[1] * e[1], 2.0 * e[0] * e[1])
            st(_IDX[2 ** b], e)
        for xv in _LO_SET:
            if xv == 0 or (xv & (xv - 1)) == 0:
                continue
            low = xv & (-xv)
            st(_IDX[xv], cmul(ld(_IDX[xv - low]), ld(_IDX[low])))
        st(_hi_idx(0, 0), (P_scr[2, prow, lanes], P_scr[3, prow, lanes]))
        for i in range(1, 16):
            low = i & (-i)
            st(_hi_idx(0, i), cmul(ld(_hi_idx(0, i - low)), ld(_IDX[16 * low])))

        def h_of(xv):
            if xv < 256:
                return _hi_idx(0, xv // 16)
            if xv < 512:
                return _hi_idx(1, (xv - 256) // 32)
            return _hi_idx(2, (xv - 512) // 64)

        for r in (1, 2, 3):
            base = 128 << r
            st16 = 16 << r
            for i in range(8):
                st(_hi_idx(r, i), cmul(ld(h_of(st16 * i)), ld(_IDX[base])))
        return carry

    jax.lax.fori_loop(0, NG * (NST // 8), tables_slice, 0)

    def kgen_unit(lg, r, ia, jh, A=4, never=None):
        step = 1 << r
        B = 8 if r == 0 else 9
        lidx = [jnp.where(jh == 0, _IDX[step * j], _IDX[step * (8 + j)]) for j in range(B)]
        hidx = [_hi_idx(r, 0) + A * ia + a for a in range(A)]

        def tl(e, s):
            return T[lg, pl.ds(pl.multiple_of(e * NST + s * 8, 8), 8), :]

        accs = [[None] * B for _ in range(A)]
        for s in range(NST // 8):
            hs = [(tl(2 * h, s), tl(2 * h + 1, s)) for h in hidx]
            for q in range(B):
                lr = tl(2 * lidx[q], s)
                li = tl(2 * lidx[q] + 1, s)
                for a in range(A):
                    t = hs[a][0] * lr - hs[a][1] * li
                    accs[a][q] = t if s == 0 else accs[a][q] + t
        if never is None:
            never = jh < 0
        accs = [[jnp.where(never, accs[0][0], accs[a][q]) for q in range(B)] for a in range(A)]
        base = 0 if r == 0 else (128 << r)
        pat = _rows_pattern(step, 8 * step)
        for a in range(A):
            rows = [jnp.sum(v, axis=0, keepdims=True) for v in accs[a]]
            l0 = pl.multiple_of(base + 16 * step * (A * ia + a) + 8 * step * jh, 8)
            Ks[lg, pl.ds(l0, 8 * step), :] = _assemble(rows, pat)

    k_scr[0:256, :] = jnp.zeros((256, DM), bf)
    vT_scr[:, 0:256] = jnp.zeros((DM, 256), bf)
    in_copies[0].wait()
    in_copies[1].wait()

    def proj_chunk(c):
        rows = pl.ds(pl.multiple_of(c * TQ, TQ), TQ)
        prow = pl.ds(pl.multiple_of(256 + c * TQ, TQ), TQ)
        xc = x_ref[rows, :]
        qkv = jnp.dot(xc, wqkv_ref[...], preferred_element_type=f32)
        q_scr[rows, :] = (qkv[:, :DM] * (DH ** -0.5 * LOG2E)).astype(bf)
        k_scr[prow, :] = qkv[:, DM:2 * DM].astype(bf)
        vT_scr[:, prow] = qkv[:, 2 * DM:].T.astype(bf)
        v8 = qkv[TQ - 8:TQ, 0:128]
        for t in range(1, 12):
            v8 = v8 + qkv[TQ - 8:TQ, t * 128:(t + 1) * 128]
        return (v8 > 0.0) & (v8 < 0.0)

    def kproj(i, carry):
        nv = proj_chunk(i)
        lg = i // 4
        for e in range(2):
            for a2 in range(2):
                kgen_unit(lg, 0, 2 * (i % 4) + a2, e, A=2, never=nv)
        for r in (1, 2, 3):
            for a2 in range(2):
                kgen_unit(lg, r, 2 * ((i // 2) % 2) + a2, i % 2, A=2, never=nv)
        return carry

    jax.lax.fori_loop(0, NQ, kproj, 0)
    CH = 256

    u32t = jnp.uint32
    row = jax.lax.broadcasted_iota(jnp.int32, (TQ, TQ), 0)
    col = jax.lax.broadcasted_iota(jnp.int32, (TQ, TQ), 1)
    tri = row <= col
    r2 = jax.lax.broadcasted_iota(jnp.int32, (TQ // 2, TQ), 0)
    c2 = jax.lax.broadcasted_iota(jnp.int32, (TQ // 2, TQ), 1)
    tri_bits = (jnp.where(2 * r2 <= c2, jnp.uint32(0xFFFF), jnp.uint32(0)) |
                jnp.where(2 * r2 + 1 <= c2, jnp.uint32(0xFFFF0000), jnp.uint32(0)))
    lane64 = c2 // DH
    NEG = -1e9 * LOG2E

    def qk_unit(i, g, slot, nvalid=3):
        r0 = pl.multiple_of(i * TQ, TQ)
        q_u = pltpu.bitcast(q_scr[pl.ds(r0, TQ), g * 128:(g + 1) * 128], u32t)
        k_rows = k_scr[pl.ds(r0, 3 * TQ), g * 128:(g + 1) * 128]
        for hh in range(8):
            qm = pltpu.bitcast(jnp.where(lane64 == hh, q_u, jnp.uint32(0)), bf)
            ST = jax.lax.dot_general(k_rows, qm, (((1,), (1,)), ((), ())), preferred_element_type=f32)
            U, M, Dg = ST[0:TQ], ST[TQ:2 * TQ], ST[2 * TQ:3 * TQ]
            if nvalid < 3:
                U = jnp.full((TQ, TQ), NEG, f32)
            if nvalid < 2:
                M = jnp.full((TQ, TQ), NEG, f32)
            C = jnp.where(tri, Dg, U)
            S_scr[slot, hh, 0:TQ, :] = C
            S_scr[slot, hh, TQ:2 * TQ, :] = M
            Mx_scr[slot, hh] = jnp.max(jnp.maximum(C, M).reshape(TQ // 8, 8, TQ), axis=0)

    def softpv_unit(i, g, slot):
        r0 = pl.multiple_of(i * TQ, TQ)
        for hh in range(8):
            h = g * 8 + hh
            m = jnp.max(Mx_scr[slot, hh], axis=0, keepdims=True)
            P = jnp.exp2(S_scr[slot, hh] - m)
            l = jnp.sum(P, axis=0, keepdims=True)
            Pb = P.astype(bf)
            PCu = pltpu.bitcast(Pb[0:TQ], u32t)
            PD = pltpu.bitcast(PCu & tri_bits, bf)
            PU = pltpu.bitcast(PCu & ~tri_bits, bf)
            PT = jnp.concatenate([PU, Pb[TQ:2 * TQ], PD], axis=0)
            vh = vT_scr[h * DH:(h + 1) * DH, pl.ds(r0, 3 * TQ)]
            oT = jnp.dot(vh, PT, preferred_element_type=f32)
            OT_scr[h * DH:(h + 1) * DH, pl.ds(r0, TQ)] = (oT / l).astype(bf)

    def qblock(i, nv, nv_next, inext):
        qk_unit(i, 1, 1, nv)
        softpv_unit(i, 0, 0)
        qk_unit(i, 2, 0, nv)
        softpv_unit(i, 1, 1)
        qk_unit(i, 3, 1, nv)
        softpv_unit(i, 2, 0)
        qk_unit(inext, 0, 0, nv_next)
        softpv_unit(i, 3, 1)

    def qblock_loop(i, carry):
        qblock(i, 3, 3, jnp.minimum(i + 1, NQ - 1))
        return carry

    qk_unit(0, 0, 0, 1)
    qblock(0, 1, 2, 1)
    qblock(1, 2, 3, 2)
    jax.lax.fori_loop(2, NQ, qblock_loop, 0)

    in_copies[7].wait()
    out_copies = []
    for c in range(S // CH):
        o = jax.lax.dot_general(OT_scr[:, c * CH:(c + 1) * CH], wo_ref[...], (((0,), (0,)), ((), ())),
                                preferred_element_type=f32)
        outA[c * CH:(c + 1) * CH, :] = o.astype(bf)
        cp = pltpu.make_async_copy(outA.at[c * CH:(c + 1) * CH, :], out_hbm.at[c * CH:(c + 1) * CH, 0:DM], out_sems.at[c])
        cp.start()
        out_copies.append(cp)

    in_copies[2].wait()
    in_copies[3].wait()
    for g in range(NG):
        u32[g] = u_ref[:, g * 128:(g + 1) * 128].astype(f32)
    zero8 = jnp.zeros((8, 128), f32)

    def s1(j, carry):
        for g in range(NG):
            for sig in range(2):
                src = u32 if sig == 0 else Ks
                X = [src[g, pl.ds(pl.multiple_of(64 * n1 + 8 * j, 8), 8), :] for n1 in range(32)]
                W = [_transpose8(X[8 * a:8 * a + 8]) for a in range(4)]
                for t in range(8):
                    n2 = 8 * j + t
                    xs = jnp.concatenate([W[a][t] for a in range(4)], axis=0)
                    F = F1_ref[n2]
                    r0 = pl.multiple_of(n2 * R1, 8)
                    if sig == 0:
                        xu = xs.astype(bf)
                        T[g, pl.ds(_BU0 + r0, R1), :] = jnp.dot(F[:, 0:64], jnp.concatenate([xu, xu], axis=0),
                                                                preferred_element_type=f32)
                    else:
                        T[g, pl.ds(_BK0 + r0, R1), :] = jnp.dot(F, _split3(xs), preferred_element_type=f32)
            for t in range(8):
                c0 = pl.multiple_of((8 * j + t) * RC, 8)
                Cs[g, pl.ds(c0 + 32, 8), :] = zero8
                Cs[g, pl.ds(c0 + 72, 8), :] = zero8
        return carry

    jax.lax.fori_loop(0, 8, s1, 0)

    def s2(k1, carry):
        F2 = F2_ref[...]
        F2i = F2i_ref[...]
        Xs = []
        for g in range(NG):
            iu = jnp.concatenate([T[g, pl.ds(_BU0 + k1, 64, stride=R1), :],
                                  T[g, pl.ds(_BU0 + 33 + k1, 64, stride=R1), :]], axis=0)
            Xu = jnp.dot(F2, _split3(iu), preferred_element_type=f32)
            ik = jnp.concatenate([T[g, pl.ds(_BK0 + k1, 64, stride=R1), :],
                                  T[g, pl.ds(_BK0 + 33 + k1, 64, stride=R1), :]], axis=0)
            Xk = jnp.dot(F2, _split3(ik), preferred_element_type=f32)
            Xs.append((Xu, Xk))
        for g in range(NG):
            Xu, Xk = Xs[g]
            ur, ui, kr, ki = Xu[0:64], Xu[64:128], Xk[0:64], Xk[64:128]
            Y = jnp.concatenate([ur * kr - ui * ki, ur * ki + ui * kr], axis=0)
            Cv = jnp.dot(F2i, _split3(Y), preferred_element_type=f32)
            Cs[g, pl.ds(k1, 64, stride=RC), :] = Cv[0:64]
            Cs[g, pl.ds(40 + k1, 64, stride=RC), :] = Cv[64:128]
        return carry

    in_copies[4].wait()
    in_copies[5].wait()
    jax.lax.fori_loop(0, 33, s2, 0, unroll=11)

    def s3(n2, carry):
        Gm = G_ref[n2]
        for g in range(NG):
            inp = Cs[g, pl.ds(pl.multiple_of(n2 * RC, 8), RC), :]
            Ks[g, pl.ds(n2, 32, stride=64), :] = jnp.dot(Gm, _split3(inp), preferred_element_type=f32)
        return carry

    in_copies[6].wait()
    jax.lax.fori_loop(0, 64, s3, 0, unroll=8)

    for g in range(NG):
        yb = Ks[g].astype(bf).astype(f32)
        sk = (u_ref[:, g * 128:(g + 1) * 128].astype(f32) * dsk_ref[:, g * 128:(g + 1) * 128].astype(f32)).astype(bf).astype(f32)
        outB[:, g * 128:(g + 1) * 128] = (yb + sk).astype(bf)
        cp = pltpu.make_async_copy(outB.at[:, g * 128:(g + 1) * 128],
                                   out_hbm.at[:, DM + g * 128:DM + (g + 1) * 128], out_sems.at[S // CH + g])
        cp.start()
        out_copies.append(cp)
    for cp in out_copies:
        cp.wait()


@jax.jit
def pallas_concat_heads__sliding_block__ssm_conv_s4__prompt_kernel(
    A_x: jax.Array,
    A_wqkv: jax.Array,
    A_wo: jax.Array,
    B_u: jax.Array,
    B_A_re: jax.Array,
    B_A_im: jax.Array,
    B_B_re: jax.Array,
    B_B_im: jax.Array,
    B_C_re: jax.Array,
    B_C_im: jax.Array,
    B_log_dt: jax.Array,
    B_Dskip: jax.Array,
):
    F1, F2, F2i, G = [jnp.asarray(c) for c in _DFT_CONSTS]
    out = pl.pallas_call(
        _kernel,
        out_shape=jax.ShapeDtypeStruct((S, 2 * DM), bf),
        in_specs=[pl.BlockSpec(memory_space=pl.ANY)] * 4 + [pl.BlockSpec(memory_space=pltpu.VMEM)] * 8
                 + [pl.BlockSpec(memory_space=pl.ANY)] * 4,
        out_specs=pl.BlockSpec(memory_space=pl.ANY),
        scratch_shapes=[
            pltpu.VMEM((S, DM), bf),
            pltpu.VMEM((S + 256, DM), bf),
            pltpu.VMEM((DM, S + 256), bf),
            pltpu.VMEM((DM, S), bf),
            pltpu.VMEM((2, 8, 2 * TQ, TQ), f32),
            pltpu.VMEM((2, 8, 8, TQ), f32),
            pltpu.VMEM((NG, _T_ROWS, 128), f32),
            pltpu.VMEM((4, NST, DM), f32),
            pltpu.VMEM((NG, S, 128), f32),
            pltpu.VMEM((NG, S, 128), f32),
            pltpu.VMEM((NG, 64 * RC, 128), f32),
            pltpu.VMEM((S, DM), bf),
            pltpu.VMEM((DM, 3 * DM), bf),
            pltpu.VMEM((DM, DM), bf),
            pltpu.VMEM((S, DM), bf),
            pltpu.VMEM(_DFT_CONSTS[0].shape, bf),
            pltpu.VMEM(_DFT_CONSTS[1].shape, bf),
            pltpu.VMEM(_DFT_CONSTS[2].shape, bf),
            pltpu.VMEM(_DFT_CONSTS[3].shape, bf),
            pltpu.VMEM((S, DM), bf),
            pltpu.VMEM((S, DM), bf),
            pltpu.SemaphoreType.DMA((8,)),
            pltpu.SemaphoreType.DMA((S // 256 + NG,)),
        ],
        compiler_params=pltpu.CompilerParams(vmem_limit_bytes=120 * 1024 * 1024),
    )(A_x.reshape(S, DM), A_wqkv, A_wo, B_u.reshape(S, DM),
      B_A_re, B_A_im, B_B_re, B_B_im, B_C_re, B_C_im,
      B_log_dt.reshape(1, DM), B_Dskip.reshape(1, DM), F1, F2, F2i, G)
    return out.reshape(1, S, 2 * DM)
```

```python
import jax
import jax.numpy as jnp
import numpy as np
import ml_dtypes
import jax.experimental.pallas as pl
import jax.experimental.pallas.tpu as pltpu

f32 = jnp.float32
bf = jnp.bfloat16

S = 2048
DM = 512
DH = 16
LOG2E = 1.4426950408889634
TQ = 128
NQ = S // TQ
NST = 128
NF = 2 * S
NG = DM // 128
R1 = 72
RC = 80

_LO_SET = list(range(16)) + list(range(16, 32, 2)) + list(range(32, 64, 4)) + list(range(64, 128, 8))
_IDX = {x: i for i, x in enumerate(_LO_SET)}
_NLO = len(_LO_SET)
_NT = _NLO + 40
for _k, _x in enumerate([128, 256, 512, 1024]):
    _IDX[_x] = _NT + _k
_NTALL = _NT + 4
_ANCH = (0, 4, 8)


def _hi_idx(r, i):
    return _NLO + [0, 16, 24, 32][r] + i


def _rows_pattern(step, nrows):
    out = []
    for rho in range(nrows):
        q, rem = divmod(rho, step)
        if 2 * rem < step:
            v = q
        elif 2 * rem > step:
            v = q + 1
        else:
            v = q if q % 2 == 0 else q + 1
        out.append(v)
    return out


def _assemble(rows, pat):
    pieces = []
    k = 0
    while k < len(pat):
        k2 = k
        while k2 < len(pat) and pat[k2] == pat[k]:
            k2 += 1
        pieces.append(jnp.broadcast_to(rows[pat[k]], (k2 - k, 128)) if k2 - k > 1 else rows[pat[k]])
        k = k2
    return jnp.concatenate(pieces, axis=0)


def _split_np(F):
    Fh = F.astype(np.float32).astype(ml_dtypes.bfloat16)
    Fl = (F - Fh.astype(np.float64)).astype(np.float32).astype(ml_dtypes.bfloat16)
    return Fh, Fl


def _make_dft_consts():
    k1 = np.arange(33)
    F1 = np.zeros((64, R1, 96), ml_dtypes.bfloat16)
    G = np.zeros((64, 32, 3 * RC), ml_dtypes.bfloat16)
    for n2 in range(64):
        n = 64 * np.arange(32) + n2
        ph = -2 * np.pi * np.outer(k1, n) / NF
        M = np.zeros((R1, 32))
        M[0:33] = np.cos(ph)
        M[33:66] = np.sin(ph)
        h, l = _split_np(M)
        F1[n2] = np.concatenate([h, l, h], 1)
        ph = 2 * np.pi * np.outer(n, k1) / NF
        w = np.full(33, 2.0)
        w[0] = 1
        w[32] = 1
        w /= NF
        M = np.zeros((32, RC))
        M[:, 0:33] = w * np.cos(ph)
        M[:, 40:73] = -w * np.sin(ph)
        h, l = _split_np(M)
        G[n2] = np.concatenate([h, l, h], 1)
    n2k2 = np.outer(np.arange(64), np.arange(64))
    C64 = np.cos(2 * np.pi * n2k2 / 64)
    S64 = -np.sin(2 * np.pi * n2k2 / 64)
    h, l = _split_np(np.block([[C64, -S64], [S64, C64]]))
    F2 = np.concatenate([h, l, h], 1)
    h, l = _split_np(np.block([[C64, S64], [-S64, C64]]))
    F2i = np.concatenate([h, l, h], 1)
    return F1, F2, F2i, G


_DFT_CONSTS = _make_dft_consts()


def _sincos(x):
    k = jnp.floor(x * 0.6366197723675814 + 0.5)
    r = ((x - k * 1.5703125) - k * 4.837512969970703125e-4) - k * 7.54978995489188216e-8
    z = r * r
    s = ((-1.9515295891e-4 * z + 8.3321608736e-3) * z - 1.6666654611e-1) * z * r + r
    c = ((2.443315711809948e-5 * z - 1.388731625493765e-3) * z + 4.166664568298827e-2) * z * z - 0.5 * z + 1.0
    q = k.astype(jnp.int32)
    swap = (q & 1) != 0
    sn = jnp.where(swap, c, s)
    cs = jnp.where(swap, s, c)
    sn = jnp.where((q & 2) != 0, -sn, sn)
    cs = jnp.where(((q + 1) & 2) != 0, -cs, cs)
    return sn, cs


def _split3(x):
    xh = x.astype(bf)
    xl = (x - xh.astype(f32)).astype(bf)
    return jnp.concatenate([xh, xh, xl], axis=0)


def _transpose8(vs):
    sub = jax.lax.broadcasted_iota(jnp.int32, (8, 128), 0)
    for sh in (4, 2, 1):
        low = (sub & sh) == 0
        new = list(vs)
        for a in range(8):
            if a & sh == 0:
                lo, hi = vs[a], vs[a + sh]
                new[a] = jnp.where(low, lo, pltpu.roll(hi, sh, 0))
                new[a + sh] = jnp.where(low, pltpu.roll(lo, 8 - sh, 0), hi)
        vs = new
    return vs


_T_ROWS = 2 * _NTALL * NST
_BU0 = 0
_BK0 = _BU0 + 64 * R1
assert _BK0 + 64 * R1 <= _T_ROWS


def _kernel(x_hbm, wqkv_hbm, wo_hbm, u_hbm, are_ref, aim_ref, bre_ref, bim_ref, cre_ref, cim_ref,
            ldt_ref, dsk_ref, F1_hbm, F2_hbm, F2i_hbm, G_hbm,
            out_hbm,
            q_scr, k_scr, vT_scr, OT_scr, S_scr, Mx_scr, T, P_scr, Ks, u32, Cs,
            x_ref, wqkv_ref, wo_ref, u_ref, F1_ref, F2_ref, F2i_ref, G_ref, outA, outB, in_sems, out_sems):
    in_pairs = [(x_hbm, x_ref), (wqkv_hbm, wqkv_ref), (u_hbm, u_ref), (F1_hbm, F1_ref), (F2_hbm, F2_ref),
                (F2i_hbm, F2i_ref), (G_hbm, G_ref), (wo_hbm, wo_ref)]
    in_copies = [pltpu.make_async_copy(src, dst, in_sems.at[j]) for j, (src, dst) in enumerate(in_pairs)]
    for cp in in_copies:
        cp.start()

    dt = jnp.exp(ldt_ref[...].astype(f32)).astype(bf).astype(f32)

    def tr(ref):
        return ref[...].astype(f32).T

    ar = tr(are_ref) * dt
    ai = tr(aim_ref) * dt
    dBr = tr(bre_ref) * dt
    dBi = tr(bim_ref) * dt
    Cr = tr(cre_ref)
    Ci = tr(cim_ref)
    P_scr[0] = ar
    P_scr[1] = ai
    P_scr[2] = Cr * dBr - Ci * dBi
    P_scr[3] = Cr * dBi + Ci * dBr

    def tables_slice(it, carry):
        lg = it // (NST // 8)
        s = it % (NST // 8)
        lanes = pl.ds(pl.multiple_of(lg * 128, 128), 128)
        prow = pl.ds(pl.multiple_of(s * 8, 8), 8)

        def trow(e):
            return pl.ds(pl.multiple_of(e * NST + s * 8, 8), 8)

        def st(idx, v):
            T[lg, trow(2 * idx), :] = v[0]
            T[lg, trow(2 * idx + 1), :] = v[1]

        def ld(idx):
            return T[lg, trow(2 * idx), :], T[lg, trow(2 * idx + 1), :]

        def cmul(a, b):
            return a[0] * b[0] - a[1] * b[1], a[0] * b[1] + a[1] * b[0]

        ar_s = P_scr[0, prow, lanes]
        ai_s = P_scr[1, prow, lanes]
        st(_IDX[0], (jnp.ones((8, 128), f32), jnp.zeros((8, 128), f32)))
        e = None
        for b in range(11):
            if b in _ANCH:
                xx = float(2 ** b)
                m = jnp.exp(ar_s * xx)
                th = ai_s * xx
                sn, cs = _sincos(th)
                e = (m * cs, m * sn)
            else:
                e = (e[0] * e[0] - e[1] * e[1], 2.0 * e[0] * e[1])
            st(_IDX[2 ** b], e)
        for xv in _LO_SET:
            if xv == 0 or (xv & (xv - 1)) == 0:
                continue
            low = xv & (-xv)
            st(_IDX[xv], cmul(ld(_IDX[xv - low]), ld(_IDX[low])))
        st(_hi_idx(0, 0), (P_scr[2, prow, lanes], P_scr[3, prow, lanes]))
        for i in range(1, 16):
            low = i & (-i)
            st(_hi_idx(0, i), cmul(ld(_hi_idx(0, i - low)), ld(_IDX[16 * low])))

        def h_of(xv):
            if xv < 256:
                return _hi_idx(0, xv // 16)
            if xv < 512:
                return _hi_idx(1, (xv - 256) // 32)
            return _hi_idx(2, (xv - 512) // 64)

        for r in (1, 2, 3):
            base = 128 << r
            st16 = 16 << r
            for i in range(8):
                st(_hi_idx(r, i), cmul(ld(h_of(st16 * i)), ld(_IDX[base])))
        return carry

    jax.lax.fori_loop(0, NG * (NST // 8), tables_slice, 0)

    def kgen_acc(lg, r, ia, jh, A):
        step = 1 << r
        B = 8 if r == 0 else 9
        lidx = [jnp.where(jh == 0, _IDX[step * j], _IDX[step * (8 + j)]) for j in range(B)]
        hidx = [_hi_idx(r, 0) + A * ia + a for a in range(A)]

        def tl(e, s):
            return T[lg, pl.ds(pl.multiple_of(e * NST + s * 8, 8), 8), :]

        accs = [[None] * B for _ in range(A)]
        for s in range(NST // 8):
            hs = [(tl(2 * h, s), tl(2 * h + 1, s)) for h in hidx]
            for q in range(B):
                lr = tl(2 * lidx[q], s)
                li = tl(2 * lidx[q] + 1, s)
                for a in range(A):
                    t = hs[a][0] * lr - hs[a][1] * li
                    accs[a][q] = t if s == 0 else accs[a][q] + t
        return accs

    def kgen_sink(lg, r, ia, jh, A, accs, never):
        step = 1 << r
        B = len(accs[0])
        accs = [[jnp.where(never, accs[0][0], accs[a][q]) for q in range(B)] for a in range(A)]
        base = 0 if r == 0 else (128 << r)
        pat = _rows_pattern(step, 8 * step)
        for a in range(A):
            rows = [jnp.sum(v, axis=0, keepdims=True) for v in accs[a]]
            l0 = pl.multiple_of(base + 16 * step * (A * ia + a) + 8 * step * jh, 8)
            Ks[lg, pl.ds(l0, 8 * step), :] = _assemble(rows, pat)

    def kgen_units(i):
        lg = i // 4
        us = [(lg, 0, 2 * (i % 4) + a2, e) for e in range(2) for a2 in range(2)]
        us += [(lg, r, 2 * ((i // 2) % 2) + a2, i % 2) for r in (1, 2, 3) for a2 in range(2)]
        return us

    k_scr[0:256, :] = jnp.zeros((256, DM), bf)
    vT_scr[:, 0:256] = jnp.zeros((DM, 256), bf)
    in_copies[0].wait()
    in_copies[1].wait()

    def proj_chunk(c):
        rows = pl.ds(pl.multiple_of(c * TQ, TQ), TQ)
        prow = pl.ds(pl.multiple_of(256 + c * TQ, TQ), TQ)
        xc = x_ref[rows, :]
        qkv = jnp.dot(xc, wqkv_ref[...], preferred_element_type=f32)
        q_scr[rows, :] = (qkv[:, :DM] * (DH ** -0.5 * LOG2E)).astype(bf)
        k_scr[prow, :] = qkv[:, DM:2 * DM].astype(bf)
        vT_scr[:, prow] = qkv[:, 2 * DM:].T.astype(bf)
        v8 = qkv[TQ - 8:TQ, 0:128]
        for t in range(1, 12):
            v8 = v8 + qkv[TQ - 8:TQ, t * 128:(t + 1) * 128]
        return v8

    def kgen_part(i, mxu_work):
        us = kgen_units(i)
        accs = [kgen_acc(*u, 2) for u in us]
        mk = mxu_work()
        never = (mk > 0.0) & (mk < 0.0)
        for u, ac in zip(us, accs):
            kgen_sink(*u, 2, ac, never)

    kgen_part(0, lambda: proj_chunk(0))
    CH = 256

    u32t = jnp.uint32
    row = jax.lax.broadcasted_iota(jnp.int32, (TQ, TQ), 0)
    col = jax.lax.broadcasted_iota(jnp.int32, (TQ, TQ), 1)
    tri = row <= col
    r2 = jax.lax.broadcasted_iota(jnp.int32, (TQ // 2, TQ), 0)
    c2 = jax.lax.broadcasted_iota(jnp.int32, (TQ // 2, TQ), 1)
    tri_bits = (jnp.where(2 * r2 <= c2, jnp.uint32(0xFFFF), jnp.uint32(0)) |
                jnp.where(2 * r2 + 1 <= c2, jnp.uint32(0xFFFF0000), jnp.uint32(0)))
    lane64 = c2 // DH
    NEG = -1e9 * LOG2E

    def qk_unit(i, g, slot, nvalid=3):
        r0 = pl.multiple_of(i * TQ, TQ)
        q_u = pltpu.bitcast(q_scr[pl.ds(r0, TQ), g * 128:(g + 1) * 128], u32t)
        k_rows = k_scr[pl.ds(r0, 3 * TQ), g * 128:(g + 1) * 128]
        for hh in range(8):
            qm = pltpu.bitcast(jnp.where(lane64 == hh, q_u, jnp.uint32(0)), bf)
            ST = jax.lax.dot_general(k_rows, qm, (((1,), (1,)), ((), ())), preferred_element_type=f32)
            U, M, Dg = ST[0:TQ], ST[TQ:2 * TQ], ST[2 * TQ:3 * TQ]
            if nvalid < 3:
                U = jnp.full((TQ, TQ), NEG, f32)
            if nvalid < 2:
                M = jnp.full((TQ, TQ), NEG, f32)
            C = jnp.where(tri, Dg, U)
            S_scr[slot, hh, 0:TQ, :] = C
            S_scr[slot, hh, TQ:2 * TQ, :] = M
            Mx_scr[slot, hh] = jnp.max(jnp.maximum(C, M).reshape(TQ // 8, 8, TQ), axis=0)

    def softpv_unit(i, g, slot):
        r0 = pl.multiple_of(i * TQ, TQ)
        for hh in range(8):
            h = g * 8 + hh
            m = jnp.max(Mx_scr[slot, hh], axis=0, keepdims=True)
            P = jnp.exp2(S_scr[slot, hh] - m)
            l = jnp.sum(P, axis=0, keepdims=True)
            Pb = P.astype(bf)
            PCu = pltpu.bitcast(Pb[0:TQ], u32t)
            PD = pltpu.bitcast(PCu & tri_bits, bf)
            PU = pltpu.bitcast(PCu & ~tri_bits, bf)
            PT = jnp.concatenate([PU, Pb[TQ:2 * TQ], PD], axis=0)
            vh = vT_scr[h * DH:(h + 1) * DH, pl.ds(r0, 3 * TQ)]
            oT = jnp.dot(vh, PT, preferred_element_type=f32)
            OT_scr[h * DH:(h + 1) * DH, pl.ds(r0, TQ)] = (oT / l).astype(bf)
        return oT[0:8]

    def qblock(i, nv, nv_next, inext):
        qk_unit(i, 1, 1, nv)
        softpv_unit(i, 0, 0)
        qk_unit(i, 2, 0, nv)
        softpv_unit(i, 1, 1)
        qk_unit(i, 3, 1, nv)
        softpv_unit(i, 2, 0)
        qk_unit(inext, 0, 0, nv_next)
        return softpv_unit(i, 3, 1)

    def mega(i, nv, nv_next):
        kgen_part(i, lambda: proj_chunk(i) + qblock(i - 1, nv, nv_next, i))

    def mega_loop(i, carry):
        mega(i, 3, 3)
        return carry

    qk_unit(0, 0, 0, 1)
    mega(1, 1, 2)
    mega(2, 2, 3)
    jax.lax.fori_loop(3, NQ, mega_loop, 0)
    qblock(NQ - 1, 3, 3, NQ - 1)

    in_copies[7].wait()
    out_copies = []
    for c in range(S // CH):
        o = jax.lax.dot_general(OT_scr[:, c * CH:(c + 1) * CH], wo_ref[...], (((0,), (0,)), ((), ())),
                                preferred_element_type=f32)
        outA[c * CH:(c + 1) * CH, :] = o.astype(bf)
        cp = pltpu.make_async_copy(outA.at[c * CH:(c + 1) * CH, :], out_hbm.at[c * CH:(c + 1) * CH, 0:DM], out_sems.at[c])
        cp.start()
        out_copies.append(cp)

    in_copies[2].wait()
    in_copies[3].wait()
    for g in range(NG):
        u32[g] = u_ref[:, g * 128:(g + 1) * 128].astype(f32)
    zero8 = jnp.zeros((8, 128), f32)

    def s1(j, carry):
        for g in range(NG):
            for sig in range(2):
                src = u32 if sig == 0 else Ks
                X = [src[g, pl.ds(pl.multiple_of(64 * n1 + 8 * j, 8), 8), :] for n1 in range(32)]
                W = [_transpose8(X[8 * a:8 * a + 8]) for a in range(4)]
                for t in range(8):
                    n2 = 8 * j + t
                    xs = jnp.concatenate([W[a][t] for a in range(4)], axis=0)
                    F = F1_ref[n2]
                    r0 = pl.multiple_of(n2 * R1, 8)
                    if sig == 0:
                        xu = xs.astype(bf)
                        T[g, pl.ds(_BU0 + r0, R1), :] = jnp.dot(F[:, 0:64], jnp.concatenate([xu, xu], axis=0),
                                                                preferred_element_type=f32)
                    else:
                        T[g, pl.ds(_BK0 + r0, R1), :] = jnp.dot(F, _split3(xs), preferred_element_type=f32)
            for t in range(8):
                c0 = pl.multiple_of((8 * j + t) * RC, 8)
                Cs[g, pl.ds(c0 + 32, 8), :] = zero8
                Cs[g, pl.ds(c0 + 72, 8), :] = zero8
        return carry

    jax.lax.fori_loop(0, 8, s1, 0)

    def s2(k1, carry):
        F2 = F2_ref[...]
        F2i = F2i_ref[...]
        Xs = []
        for g in range(NG):
            iu = jnp.concatenate([T[g, pl.ds(_BU0 + k1, 64, stride=R1), :],
                                  T[g, pl.ds(_BU0 + 33 + k1, 64, stride=R1), :]], axis=0)
            Xu = jnp.dot(F2, _split3(iu), preferred_element_type=f32)
            ik = jnp.concatenate([T[g, pl.ds(_BK0 + k1, 64, stride=R1), :],
                                  T[g, pl.ds(_BK0 + 33 + k1, 64, stride=R1), :]], axis=0)
            Xk = jnp.dot(F2, _split3(ik), preferred_element_type=f32)
            Xs.append((Xu, Xk))
        for g in range(NG):
            Xu, Xk = Xs[g]
            ur, ui, kr, ki = Xu[0:64], Xu[64:128], Xk[0:64], Xk[64:128]
            Y = jnp.concatenate([ur * kr - ui * ki, ur * ki + ui * kr], axis=0)
            Cv = jnp.dot(F2i, _split3(Y), preferred_element_type=f32)
            Cs[g, pl.ds(k1, 64, stride=RC), :] = Cv[0:64]
            Cs[g, pl.ds(40 + k1, 64, stride=RC), :] = Cv[64:128]
        return carry

    in_copies[4].wait()
    in_copies[5].wait()
    jax.lax.fori_loop(0, 33, s2, 0, unroll=11)

    def s3(n2, carry):
        Gm = G_ref[n2]
        for g in range(NG):
            inp = Cs[g, pl.ds(pl.multiple_of(n2 * RC, 8), RC), :]
            Ks[g, pl.ds(n2, 32, stride=64), :] = jnp.dot(Gm, _split3(inp), preferred_element_type=f32)
        return carry

    in_copies[6].wait()
    jax.lax.fori_loop(0, 64, s3, 0, unroll=8)

    for g in range(NG):
        yb = Ks[g].astype(bf).astype(f32)
        sk = (u_ref[:, g * 128:(g + 1) * 128].astype(f32) * dsk_ref[:, g * 128:(g + 1) * 128].astype(f32)).astype(bf).astype(f32)
        outB[:, g * 128:(g + 1) * 128] = (yb + sk).astype(bf)
        cp = pltpu.make_async_copy(outB.at[:, g * 128:(g + 1) * 128],
                                   out_hbm.at[:, DM + g * 128:DM + (g + 1) * 128], out_sems.at[S // CH + g])
        cp.start()
        out_copies.append(cp)
    for cp in out_copies:
        cp.wait()


@jax.jit
def pallas_concat_heads__sliding_block__ssm_conv_s4__prompt_kernel(
    A_x: jax.Array,
    A_wqkv: jax.Array,
    A_wo: jax.Array,
    B_u: jax.Array,
    B_A_re: jax.Array,
    B_A_im: jax.Array,
    B_B_re: jax.Array,
    B_B_im: jax.Array,
    B_C_re: jax.Array,
    B_C_im: jax.Array,
    B_log_dt: jax.Array,
    B_Dskip: jax.Array,
):
    F1, F2, F2i, G = [jnp.asarray(c) for c in _DFT_CONSTS]
    out = pl.pallas_call(
        _kernel,
        out_shape=jax.ShapeDtypeStruct((S, 2 * DM), bf),
        in_specs=[pl.BlockSpec(memory_space=pl.ANY)] * 4 + [pl.BlockSpec(memory_space=pltpu.VMEM)] * 8
                 + [pl.BlockSpec(memory_space=pl.ANY)] * 4,
        out_specs=pl.BlockSpec(memory_space=pl.ANY),
        scratch_shapes=[
            pltpu.VMEM((S, DM), bf),
            pltpu.VMEM((S + 256, DM), bf),
            pltpu.VMEM((DM, S + 256), bf),
            pltpu.VMEM((DM, S), bf),
            pltpu.VMEM((2, 8, 2 * TQ, TQ), f32),
            pltpu.VMEM((2, 8, 8, TQ), f32),
            pltpu.VMEM((NG, _T_ROWS, 128), f32),
            pltpu.VMEM((4, NST, DM), f32),
            pltpu.VMEM((NG, S, 128), f32),
            pltpu.VMEM((NG, S, 128), f32),
            pltpu.VMEM((NG, 64 * RC, 128), f32),
            pltpu.VMEM((S, DM), bf),
            pltpu.VMEM((DM, 3 * DM), bf),
            pltpu.VMEM((DM, DM), bf),
            pltpu.VMEM((S, DM), bf),
            pltpu.VMEM(_DFT_CONSTS[0].shape, bf),
            pltpu.VMEM(_DFT_CONSTS[1].shape, bf),
            pltpu.VMEM(_DFT_CONSTS[2].shape, bf),
            pltpu.VMEM(_DFT_CONSTS[3].shape, bf),
            pltpu.VMEM((S, DM), bf),
            pltpu.VMEM((S, DM), bf),
            pltpu.SemaphoreType.DMA((8,)),
            pltpu.SemaphoreType.DMA((S // 256 + NG,)),
        ],
        compiler_params=pltpu.CompilerParams(vmem_limit_bytes=120 * 1024 * 1024),
    )(A_x.reshape(S, DM), A_wqkv, A_wo, B_u.reshape(S, DM),
      B_A_re, B_A_im, B_B_re, B_B_im, B_C_re, B_C_im,
      B_log_dt.reshape(1, DM), B_Dskip.reshape(1, DM), F1, F2, F2i, G)
    return out.reshape(1, S, 2 * DM)
```
